```python
import jax
import jax.numpy as jnp

def _softmax(x, axis=-1):
    return jax.nn.softmax(x, axis=axis)

def _gelu(x):
    return jax.nn.gelu(x, approximate=True)

def _silu(x):
    return jax.nn.silu(x)

def _sigmoid(x):
    return jax.nn.sigmoid(x)

def _layernorm(x, axis=-1, eps=1e-05):
    m = jnp.mean(x, axis=axis, keepdims=True)
    v = jnp.var(x, axis=axis, keepdims=True)
    return (x - m) / jnp.sqrt(v + eps)

def _scatter_add(tgt, idx, src, axis=0):
    return tgt.at[idx].add(src)

def _segment_sum(src, seg, n):
    return jax.ops.segment_sum(src, seg, n)

class _Rng:

    def __init__(self, key):
        self._k = key

    def _next(self):
        self._k, sub = jax.random.split(self._k)
        return sub

    def normal(self, shape):
        return jax.random.normal(self._next(), shape, dtype=jnp.bfloat16)

    def randint(self, lo, hi, shape):
        return jax.random.randint(self._next(), shape, lo, hi, dtype=jnp.int32)

    def uniform(self, shape, lo=0.0, hi=1.0):
        return jax.random.uniform(self._next(), shape, jnp.bfloat16, lo, hi)

    def permutation(self, n):
        return jax.random.permutation(self._next(), n)
kernel_name = 'adaLN_cond__ssm_conv_h3__glu_gated_bilinear__prompt'

def setup_inputs():
    _rng = _Rng(jax.random.key(int.from_bytes(__import__("os").urandom(4), "little")))
    _w = lambda a: (lambda t: t.astype(jnp.bfloat16) if jnp.issubdtype(t.dtype, jnp.floating) else t)(jnp.asarray(a))

    def _A_setup():
        B, S, D = (1, 2048, 640)
        ks = 4
        return {'q': _w((lambda *s: _rng.normal(s) * 0.05)(B, S, D)), 'k': _w((lambda *s: _rng.normal(s) * 0.05)(B, S, D)), 'v': _w((lambda *s: _rng.normal(s) * 0.05)(B, S, D)), 'shift_k': _w((lambda *s: _rng.normal(s) * 0.05)(D, ks) * 0.5), 'ssm_k': _w((lambda *s: _rng.normal(s) * 0.05)(D, S) * (1.0 / S ** 0.5)), 'ssm_D': _w((lambda *s: _rng.normal(s) * 0.05)(D))}
    _A_in = _A_setup()

    def _B_setup():
        B, S, D, F = (1, 2048, 640, 1536)
        return {'x': _w((lambda *s: _rng.normal(s) * 0.05)(B, S, D)), 'w_gate': _w((lambda *s: _rng.normal(s) * 0.05)(D, F) * D ** (-0.5)), 'w_up': _w((lambda *s: _rng.normal(s) * 0.05)(D, F) * D ** (-0.5)), 'w_down': _w((lambda *s: _rng.normal(s) * 0.05)(F, D) * F ** (-0.5))}
    _B_in = _B_setup()
    return {'A_q': _A_in['q'], 'A_k': _A_in['k'], 'A_v': _A_in['v'], 'A_shift_k': _A_in['shift_k'], 'A_ssm_k': _A_in['ssm_k'], 'A_ssm_D': _A_in['ssm_D'], 'B_x': _B_in['x'], 'B_w_gate': _B_in['w_gate'], 'B_w_up': _B_in['w_up'], 'B_w_down': _B_in['w_down'], 'c': _w((lambda *s: _rng.normal(s) * 0.05)(1, 640)), 'w_mod': _w((lambda *s: _rng.normal(s) * 0.05)(640, 6 * 640) * 640 ** (-0.5))}

def reference(A_q, A_k, A_v, A_shift_k, A_ssm_k, A_ssm_D, B_x, B_w_gate, B_w_up, B_w_down, c, w_mod):

    def _A_ref(q, k, v, shift_k, ssm_k, ssm_D):
        B, S, D = q.shape
        ks = shift_k.shape[-1]
        k_pad = jnp.pad(k, ((0, 0), (ks - 1, 0), (0, 0)))
        k_shift = jnp.zeros_like(k)
        for t in range(ks):
            k_shift = k_shift + k_pad[:, t:t + S, :] * shift_k[:, ks - 1 - t][None, None, :]
        kv = k_shift * v
        L = 2 * S
        kv_pad = jnp.pad(kv, ((0, 0), (0, S), (0, 0)))
        kf_pad = jnp.pad(ssm_k, ((0, 0), (0, S)))
        kv_f = (lambda x, axes=(-2, -1): jnp.fft.rfft2(x.astype(jnp.float32), axes=axes))(kv_pad[:, None, :, :], axes=(1, 2))
        kf_f = (lambda x, axes=(-2, -1): jnp.fft.rfft2(x.astype(jnp.float32), axes=axes))(kf_pad[:, None, :], axes=(1, 2))
        kf_f = (lambda x, *d: x.transpose(*d))(kf_f, 1, 2, 0)
        y_f = kv_f * kf_f[None, :, :, :]
        y = (lambda x, s, axes=(-2, -1): jnp.fft.irfft2(x, s=s, axes=axes).astype(jnp.bfloat16))(y_f, (1, L), axes=(1, 2))[:, 0, :S, :]
        y = y + kv * ssm_D[None, None, :]
        return q * y

    def _B_ref(x, w_gate, w_up, w_down):
        g = jnp.einsum('bsd,df->bsf', x, w_gate)
        u = jnp.einsum('bsd,df->bsf', x, w_up)
        h = g * u
        return jnp.einsum('bsf,fd->bsd', h, w_down)
    x = A_q
    mod = (_silu(c) @ w_mod).reshape(c.shape[0], 6, 1, -1)
    sa, ca, ga, sb, cb, gb = (mod[:, 0].copy(), mod[:, 1].copy(), mod[:, 2].copy(), mod[:, 3].copy(), mod[:, 4].copy(), mod[:, 5].copy())
    h = _layernorm(x, axis=-1) * (1 + ca) + sa
    x = x + ga * _A_ref(h, A_k, A_v, A_shift_k, A_ssm_k, A_ssm_D)
    h = _layernorm(x, axis=-1) * (1 + cb) + sb
    x = x + gb * _B_ref(h, B_w_gate, B_w_up, B_w_down)
    return x
```

```python
import functools

import jax
import jax.numpy as jnp
import ml_dtypes
import numpy as np
from jax import lax
import jax.experimental.pallas as pl
import jax.experimental.pallas.tpu as pltpu

S, D, F = 2048, 640, 1536
L = 256
P = S // L
N2 = L // 2
EPS = 1e-5


def _dft_consts():
    k = np.concatenate([np.arange(0, N2, 2), np.arange(1, N2, 2)])
    theta = (2 * k + 1) * np.pi / (2 * L)

    def mk(t):
        a = theta[:, None] * t[None, :]
        return np.concatenate([np.cos(a), -np.sin(a)], 0)

    n = np.arange(N2)
    fe, fo = mk(2 * n), mk(2 * n + 1)
    t = np.arange(L)
    fp = mk(t)
    fh = np.concatenate([fp, fp * ((-1.0) ** t)[None, :]], 0)
    bf = ml_dtypes.bfloat16
    f = np.concatenate([fe, fo], 0).astype(bf)
    g = (np.concatenate([fe.T, fo.T], 0) / L).astype(bf)
    return f, g, fh.astype(bf)


def _split(x_bf16):
    u = pltpu.bitcast(x_bf16, jnp.uint32)
    e = pltpu.unpack_elementwise(u, index=0, packed_dtype=jnp.bfloat16, unpacked_dtype=jnp.float32)
    o = pltpu.unpack_elementwise(u, index=1, packed_dtype=jnp.bfloat16, unpacked_dtype=jnp.float32)
    return e, o


def _ln(x):
    m = jnp.mean(x, axis=-1, keepdims=True)
    d = x - m
    v = jnp.mean(d * d, axis=-1, keepdims=True)
    return d * lax.rsqrt(v + EPS)


def _kernel(q_hbm, k_hbm, v_hbm, shk_ref, ssm_hbm, dskip_ref, wg_hbm, wu_hbm, wd_hbm,
            c_ref, wm_hbm, f_hbm, g_hbm, fh_hbm, o_hbm,
            qb, kb, vb, sb, wg, wu, wd, wm, fb, gb, fhb,
            hbuf, xbuf, wbuf, kvb, ybuf, ob,
            sem_k, sem_v, sem_s, sem_misc, sem_o):
    def cp(src, dst, sem):
        return pltpu.make_async_copy(src, dst, sem)

    rows = lambda j: pl.ds(j * L, L)
    cp_fh = cp(fh_hbm, fhb, sem_misc.at[0])
    cp_f = cp(f_hbm, fb, sem_misc.at[1])
    cp_g = cp(g_hbm, gb, sem_misc.at[2])
    cp_s = [cp(ssm_hbm.at[:, rows(j)], sb.at[:, rows(j)], sem_s.at[j]) for j in range(P)]
    cp_k = [cp(k_hbm.at[rows(j), :], kb.at[rows(j), :], sem_k.at[j]) for j in range(P)]
    cp_v = [cp(v_hbm.at[rows(j), :], vb.at[rows(j), :], sem_v.at[j]) for j in range(P)]
    cp_wm = cp(wm_hbm, wm, sem_misc.at[3])
    cp_q = cp(q_hbm, qb, sem_misc.at[4])
    cp_wg = cp(wg_hbm, wg, sem_misc.at[5])
    cp_wu = cp(wu_hbm, wu, sem_misc.at[6])
    cp_wd = cp(wd_hbm, wd, sem_misc.at[7])

    cp_fh.start()
    for j in range(P):
        cp_s[j].start()
    cp_f.start()
    for j in range(P):
        cp_k[j].start()
        cp_v[j].start()
    cp_g.start()
    cp_wm.start()
    cp_q.start()
    cp_wg.start()
    cp_wu.start()
    cp_wd.start()

    cp_fh.wait()
    fh = fhb[...]
    prev = None
    half = N2 // 2
    for m in range(P):
        cp_s[m].wait()
        hraw = lax.dot_general(fh, sb[:, rows(m)], (((1,), (1,)), ((), ())),
                               preferred_element_type=jnp.float32)
        for z in range(2):
            hr = hraw[z * L:z * L + N2]
            hi = hraw[z * L + N2:(z + 1) * L]
            if prev is not None:
                pr = prev[z * L:z * L + N2]
                pi = prev[z * L + N2:(z + 1) * L]
                hr = jnp.concatenate([hr[:half] - pi[:half], hr[half:] + pi[half:]], 0)
                hi = jnp.concatenate([hi[:half] + pr[:half], hi[half:] - pr[half:]], 0)
            hbuf[m, 3 * z + 0] = hr
            hbuf[m, 3 * z + 1] = hi
            hbuf[m, 3 * z + 2] = hr + hi
        prev = hraw

    cp_f.wait()
    w = shk_ref[...].astype(jnp.float32)
    w0, w1, w2, w3 = (w[t:t + 1] for t in range(4))
    fe = fb[0:L, :]
    fo = fb[L:2 * L, :]
    for j in range(P):
        cp_k[j].wait()
        cp_v[j].wait()
        ke, ko = _split(kb[rows(j), :])
        ve, vo = _split(vb[rows(j), :])
        if j == 0:
            pe = po = jnp.zeros((8, D), jnp.float32)
        else:
            pe, po = _split(kb[pl.ds(j * L - 16, 16), :])
        kew = jnp.concatenate([pe, ke], 0)
        kow = jnp.concatenate([po, ko], 0)
        ke1 = kew[7:7 + N2]
        ko1 = kow[7:7 + N2]
        ko2 = kow[6:6 + N2]
        kve = (w0 * ke + w1 * ko1 + w2 * ke1 + w3 * ko2) * ve
        kvo = (w0 * ko + w1 * ke + w2 * ko1 + w3 * ke1) * vo
        kve = kve.astype(jnp.bfloat16)
        kvo = kvo.astype(jnp.bfloat16)
        kvb[pl.ds(j * L, N2), :] = kve
        kvb[pl.ds(j * L + N2, N2), :] = kvo
        e = jnp.dot(fe, kve, preferred_element_type=jnp.float32)
        o = jnp.dot(fo, kvo, preferred_element_type=jnp.float32)
        for z, xz in enumerate((e + o, e - o)):
            xr, xi = xz[:N2], xz[N2:]
            xbuf[j, 3 * z + 0] = xr
            xbuf[j, 3 * z + 1] = xi
            xbuf[j, 3 * z + 2] = xr + xi

    RG = 16

    def mac_group(rg, _):
        r = pl.ds(pl.multiple_of(rg * RG, RG), RG)
        for i0 in range(0, P, 2):
            for c in range(D // 128):
                ln = slice(c * 128, (c + 1) * 128)
                z_out = {}
                for z in range(2):
                    acc = {}
                    for m in range(i0 + 2):
                        hr = hbuf[m, 3 * z + 0, r, ln]
                        hi = hbuf[m, 3 * z + 1, r, ln]
                        hs = hbuf[m, 3 * z + 2, r, ln]
                        for i in (i0, i0 + 1):
                            j = i - m
                            if j < 0:
                                continue
                            a = hr * xbuf[j, 3 * z + 0, r, ln]
                            b = hi * xbuf[j, 3 * z + 1, r, ln]
                            cc = hs * xbuf[j, 3 * z + 2, r, ln]
                            if i in acc:
                                acc[i] = (acc[i][0] + a, acc[i][1] + b, acc[i][2] + cc)
                            else:
                                acc[i] = (a, b, cc)
                    for i in (i0, i0 + 1):
                        a, b, cc = acc[i]
                        z_out[(i, z)] = (a - b, cc - a - b)
                for i in (i0, i0 + 1):
                    (pr, pi), (qr, qi) = z_out[(i, 0)], z_out[(i, 1)]
                    wbuf[i, 0, 0, r, ln] = (pr + qr).astype(jnp.bfloat16)
                    wbuf[i, 0, 1, r, ln] = (pi + qi).astype(jnp.bfloat16)
                    wbuf[i, 1, 0, r, ln] = (pr - qr).astype(jnp.bfloat16)
                    wbuf[i, 1, 1, r, ln] = (pi - qi).astype(jnp.bfloat16)
        return None

    lax.fori_loop(0, N2 // RG, mac_group, None)

    cp_g.wait()
    ge = gb[0:N2, :]
    go = gb[N2:L, :]
    for i in range(P):
        we = jnp.concatenate([wbuf[i, 0, 0], wbuf[i, 0, 1]], 0)
        wo = jnp.concatenate([wbuf[i, 1, 0], wbuf[i, 1, 1]], 0)
        ybuf[pl.ds(i * L, N2), :] = jnp.dot(ge, we, preferred_element_type=jnp.float32)
        ybuf[pl.ds(i * L + N2, N2), :] = jnp.dot(go, wo, preferred_element_type=jnp.float32)

    cp_wm.wait()
    cf = c_ref[...].astype(jnp.float32)
    sc = cf * (1.0 / (1.0 + jnp.exp(-cf)))
    sc = jnp.broadcast_to(sc, (16, D)).astype(jnp.bfloat16)
    mod = jnp.dot(sc, wm[...], preferred_element_type=jnp.float32)[0:1]
    sa, ca, ga, sb_, cb, gb_ = (mod[:, t * D:(t + 1) * D] for t in range(6))
    dskip = dskip_ref[...].astype(jnp.float32)

    cp_q.wait()
    cp_wg.wait()
    cp_wu.wait()
    cp_wd.wait()
    out_cps = []
    for i in range(P):
        qe, qo = _split(qb[rows(i), :])
        x = jnp.concatenate([qe, qo], 0)
        h = _ln(x) * (1.0 + ca) + sa
        r = ybuf[rows(i), :] + kvb[rows(i), :].astype(jnp.float32) * dskip
        x1 = x + ga * (h * r)
        h2 = (_ln(x1) * (1.0 + cb) + sb_).astype(jnp.bfloat16)
        g = jnp.dot(h2, wg[...], preferred_element_type=jnp.float32)
        u = jnp.dot(h2, wu[...], preferred_element_type=jnp.float32)
        a = (g * u).astype(jnp.bfloat16)
        mlp = jnp.dot(a, wd[...], preferred_element_type=jnp.float32)
        out = x1 + gb_ * mlp
        packed = pltpu.pack_elementwise([out[:N2], out[N2:]], packed_dtype=jnp.bfloat16)
        ob[rows(i), :] = pltpu.bitcast(packed, jnp.bfloat16)
        c_o = cp(ob.at[rows(i), :], o_hbm.at[rows(i), :], sem_o.at[i])
        c_o.start()
        out_cps.append(c_o)
    for c_o in out_cps:
        c_o.wait()


@jax.jit
def pallas_adaLN_cond__ssm_conv_h3__glu_gated_bilinear__prompt_kernel(
    A_q: jax.Array,
    A_k: jax.Array,
    A_v: jax.Array,
    A_shift_k: jax.Array,
    A_ssm_k: jax.Array,
    A_ssm_D: jax.Array,
    B_x: jax.Array,
    B_w_gate: jax.Array,
    B_w_up: jax.Array,
    B_w_down: jax.Array,
    c: jax.Array,
    w_mod: jax.Array,
):
    del B_x
    f, g, fh = _dft_consts()
    bf = jnp.bfloat16
    hbm = pl.BlockSpec(memory_space=pl.ANY)
    vmem = pl.BlockSpec(memory_space=pltpu.VMEM)
    out = pl.pallas_call(
        _kernel,
        in_specs=[hbm, hbm, hbm, vmem, hbm, vmem, hbm, hbm, hbm, vmem, hbm, hbm, hbm, hbm],
        out_specs=hbm,
        out_shape=jax.ShapeDtypeStruct((S, D), bf),
        scratch_shapes=[
            pltpu.VMEM((S, D), bf), pltpu.VMEM((S, D), bf), pltpu.VMEM((S, D), bf),
            pltpu.VMEM((D, S), bf),
            pltpu.VMEM((D, F), bf), pltpu.VMEM((D, F), bf), pltpu.VMEM((F, D), bf),
            pltpu.VMEM((D, 6 * D), bf),
            pltpu.VMEM((2 * L, N2), bf), pltpu.VMEM((L, L), bf), pltpu.VMEM((2 * L, L), bf),
            pltpu.VMEM((P, 6, N2, D), jnp.float32),
            pltpu.VMEM((P, 6, N2, D), jnp.float32),
            pltpu.VMEM((P, 2, 2, N2, D), bf),
            pltpu.VMEM((S, D), bf),
            pltpu.VMEM((S, D), jnp.float32),
            pltpu.VMEM((S, D), bf),
            pltpu.SemaphoreType.DMA((P,)), pltpu.SemaphoreType.DMA((P,)),
            pltpu.SemaphoreType.DMA((P,)), pltpu.SemaphoreType.DMA((8,)),
            pltpu.SemaphoreType.DMA((P,)),
        ],
        compiler_params=pltpu.CompilerParams(vmem_limit_bytes=110 * 1024 * 1024),
    )(A_q.reshape(S, D), A_k.reshape(S, D), A_v.reshape(S, D), A_shift_k.T, A_ssm_k,
      A_ssm_D.reshape(1, D), B_w_gate, B_w_up, B_w_down, c, w_mod, f, g, fh)
    return out.reshape(1, S, D)
```

```python
import functools

import jax
import jax.numpy as jnp
import ml_dtypes
import numpy as np
from jax import lax
import jax.experimental.pallas as pl
import jax.experimental.pallas.tpu as pltpu

CH = 1
S, D, F = 2048, 640, 1536
L = 256
P = S // L
N2 = L // 2
NC = D // 128
NF = F // 128
EPS = 1e-5
f32 = jnp.float32
bf16 = jnp.bfloat16
u32 = jnp.uint32


def _pack_rows(a):
    b = a.astype(ml_dtypes.bfloat16).view(np.uint16).astype(np.uint32)
    return b[0::2] | (b[1::2] << 16)


def _dft_consts():
    k = np.concatenate([np.arange(0, N2, 2), np.arange(1, N2, 2)])
    theta = (2 * k + 1) * np.pi / (2 * L)

    def mk(t):
        a = theta[:, None] * t[None, :]
        return np.cos(a), -np.sin(a)

    def mki(t):
        c, s = mk(t)
        return np.stack([c.reshape(N2 // 8, 8, -1), s.reshape(N2 // 8, 8, -1)], 1).reshape(2 * N2, -1)

    n = np.arange(N2)
    fe, fo = mki(2 * n), mki(2 * n + 1)
    t = np.arange(L)
    fp = mki(t)
    fh = np.concatenate([fp, fp * ((-1.0) ** t)[None, :]], 0)

    def mkg(t):
        c, s = mk(t)
        g = np.empty((N2, 2 * N2))
        g[:, 0::2] = c.T / L
        g[:, 1::2] = s.T / L
        return g

    g = np.concatenate([mkg(2 * n), mkg(2 * n + 1)], 0)
    return _pack_rows(np.concatenate([fe, fo], 0)), _pack_rows(g), _pack_rows(fh)


def _bf(x_u32):
    return pltpu.bitcast(x_u32, bf16)


def _u(x_f32):
    return pltpu.bitcast(x_f32.astype(bf16), u32)


def _lo(u):
    return pltpu.unpack_elementwise(u, index=0, packed_dtype=bf16, unpacked_dtype=f32)


def _hi(u):
    return pltpu.unpack_elementwise(u, index=1, packed_dtype=bf16, unpacked_dtype=f32)


def _pack(a, b):
    return pltpu.pack_elementwise([a, b], packed_dtype=bf16)


def _kernel(q_hbm, k_hbm, v_hbm, shk_hbm, ssm_hbm, dsk_hbm, wg_hbm, wu_hbm, wd_hbm,
            c_hbm, wm_hbm, f_hbm, g_hbm, fh_hbm, o_hbm,
            qb, kb, vb, sb, wg, wu, wd, wm, fb, gb, fhb, shk, dsk, cb_,
            hbuf, xbuf, ysave, wbuf, kvb, ybuf, x1b, h2b, ab, ob, sems):
    rows = lambda j: pl.ds(j * L, L)
    lanes = lambda c: slice(c * 128, (c + 1) * 128)
    nsem = [0]

    def cp(src, dst):
        nsem[0] += 1
        return pltpu.make_async_copy(src, dst, sems.at[nsem[0] - 1])

    cols = lambda a, n: pl.ds(a, n)
    cp_fh, cp_f, cp_g = cp(fh_hbm, fhb), cp(f_hbm, fb), cp(g_hbm, gb)
    cp_shk, cp_dsk, cp_c = cp(shk_hbm, shk), cp(dsk_hbm, dsk), cp(c_hbm, cb_)
    cp_s = [cp(ssm_hbm.at[:, rows(j)], sb.at[:, rows(j)]) for j in range(P)]
    cp_k = [cp(k_hbm.at[rows(j), :], kb.at[rows(j), :]) for j in range(P)]
    cp_v = [cp(v_hbm.at[rows(j), :], vb.at[rows(j), :]) for j in range(P)]
    cp_wm = [cp(wm_hbm.at[:, cols(t * D, D)], wm.at[:, cols(t * D, D)]) for t in range(6)]
    cp_q = [cp(q_hbm.at[rows(0), :], qb.at[rows(0), :]), cp(q_hbm.at[rows(1), :], qb.at[rows(1), :]),
            cp(q_hbm.at[pl.ds(2 * L, S - 2 * L), :], qb.at[pl.ds(2 * L, S - 2 * L), :])]
    TG = 3
    cp_wg = [cp(wg_hbm.at[:, cols(t * 128, TG * 128)], wg.at[:, cols(t * 128, TG * 128)]) for t in range(0, NF, TG)]
    cp_wu = [cp(wu_hbm.at[:, cols(t * 128, TG * 128)], wu.at[:, cols(t * 128, TG * 128)]) for t in range(0, NF, TG)]
    cp_wd = cp(wd_hbm, wd)

    order = [cp_fh, cp_s[0], cp_k[0], cp_v[0], cp_f, cp_shk]
    for j in range(1, P):
        order += [cp_s[j], cp_k[j], cp_v[j]]
    order += [cp_g, cp_c, cp_dsk, cp_wm[1], cp_wm[0], cp_wm[2], cp_q[0], cp_wm[4], cp_wm[3]]
    order += [cp_wg[0], cp_wu[0], cp_q[1]]
    for t in range(1, NF // TG):
        order += [cp_wg[t], cp_wu[t]]
    order += [cp_wd, cp_wm[5], cp_q[2]]
    for d in order:
        d.start()

    holder = {}

    def tie(x_u32, tok):
        if tok is None:
            return x_u32
        r = x_u32.shape[0]
        t8 = jnp.where(holder["never"], tok, x_u32[r - 8:, 0:128])
        bot = t8 if x_u32.shape[1] == 128 else jnp.concatenate([t8, x_u32[r - 8:, 128:]], 1)
        return jnp.concatenate([x_u32[:r - 8], bot], 0)

    def H(m, c, tok=None):
        s = sb[lanes(c), rows(m)]
        res = []
        for z in range(2):
            fh = _bf(tie(fhb[pl.ds(z * N2, N2), :], tok if z == 0 else None))
            res.append(lax.dot_general(fh, s, (((1,), (1,)), ((), ())), preferred_element_type=f32))

        def fin():
            for z in range(2):
                for g in range(N2 // 8):
                    hr = res[z][16 * g:16 * g + 8]
                    hi = res[z][16 * g + 8:16 * g + 16]
                    hbuf[m, 3 * z + 0, pl.ds(8 * g, 8), lanes(c)] = hr
                    hbuf[m, 3 * z + 1, pl.ds(8 * g, 8), lanes(c)] = hi
                    hbuf[m, 3 * z + 2, pl.ds(8 * g, 8), lanes(c)] = hr + hi
        return fin

    sub = lax.broadcasted_iota(jnp.int32, (8, 128), 0)

    def KV(j, c, tok=None):
        w0, w1, w2, w3 = (jnp.broadcast_to(holder["w"][t:t + 1, lanes(c)], (8, 128)) for t in range(4))
        ku = pltpu.bitcast(kb[rows(j), lanes(c)], u32)
        vu = pltpu.bitcast(vb[rows(j), lanes(c)], u32)
        if j == 0:
            pe1 = po1 = po2 = jnp.zeros((8, 128), f32)
        else:
            pu = pltpu.bitcast(kb[pl.ds(j * L - 16, 16), lanes(c)], u32)
            pe, po = _lo(pu), _hi(pu)
            pe1, po1, po2 = pltpu.roll(pe, 1, 0), pltpu.roll(po, 1, 0), pltpu.roll(po, 2, 0)
        kve, kvo = [], []
        for r in range(N2 // 8):
            u = ku[r * 8:(r + 1) * 8]
            ke, ko = _lo(u), _hi(u)
            re1, ro1, ro2 = pltpu.roll(ke, 1, 0), pltpu.roll(ko, 1, 0), pltpu.roll(ko, 2, 0)
            ke1 = jnp.where(sub < 1, pe1, re1)
            ko1 = jnp.where(sub < 1, po1, ro1)
            ko2 = jnp.where(sub < 2, po2, ro2)
            pe1, po1, po2 = re1, ro1, ro2
            vv = vu[r * 8:(r + 1) * 8]
            kve.append((w0 * ke + w1 * ko1 + w2 * ke1 + w3 * ko2) * _lo(vv))
            kvo.append((w0 * ko + w1 * ke + w2 * ko1 + w3 * ke1) * _hi(vv))
        pe_ = _u(jnp.concatenate(kve, 0))
        po_ = _u(jnp.concatenate(kvo, 0))
        kvb[j, 0, :, lanes(c)] = pe_
        kvb[j, 1, :, lanes(c)] = po_
        e = jnp.dot(_bf(tie(fb[0:N2, :], tok)), _bf(pe_), preferred_element_type=f32)
        o = jnp.dot(_bf(fb[N2:L, :]), _bf(po_), preferred_element_type=f32)

        def fin():
            for g in range(N2 // 8):
                er, ei = e[16 * g:16 * g + 8], e[16 * g + 8:16 * g + 16]
                or_, oi = o[16 * g:16 * g + 8], o[16 * g + 8:16 * g + 16]
                for z, (xr, xi) in enumerate(((er + or_, ei + oi), (er - or_, ei - oi))):
                    xbuf[j, 3 * z + 0, pl.ds(8 * g, 8), lanes(c)] = xr
                    xbuf[j, 3 * z + 1, pl.ds(8 * g, 8), lanes(c)] = xi
                    xbuf[j, 3 * z + 2, pl.ds(8 * g, 8), lanes(c)] = xr + xi
        return fin

    chain = []

    def MAC(p, c, rg):
        i0, i1 = 2 * p, 2 * p + 1
        r = pl.ds(rg * 8, 8)
        ln = lanes(c)
        even = rg < N2 // 16
        zs = {}
        for z in range(2):
            acc = {}
            xs_ = {}

            def X(j):
                if j not in xs_:
                    xs_[j] = tuple(xbuf[j, 3 * z + t, r, ln] for t in range(3))
                return xs_[j]

            for m in range(i1 + 1):
                hh = tuple(hbuf[m, 3 * z + t, r, ln] for t in range(3))
                if m == 0 and z == 0 and len(chain) >= CH and CH > 0:
                    hh = (jnp.where(holder["never"], pltpu.bitcast(chain[-CH], f32), hh[0]),) + hh[1:]
                for i in (i1, i0):
                    j = i - m
                    if j < 0:
                        continue
                    xx = X(j)
                    t3 = tuple(a * b for a, b in zip(hh, xx))
                    acc[i] = t3 if i not in acc else tuple(a + b for a, b in zip(acc[i], t3))
            y = {}
            for i in (i0, i1):
                a, b, cc = acc[i]
                y[i] = (a - b, cc - a - b)

            def fold(yy, pv):
                if even:
                    return yy[0] - pv[1], yy[1] + pv[0]
                return yy[0] + pv[1], yy[1] - pv[0]

            if p > 0:
                zs[(i0, z)] = fold(y[i0], (ysave[2 * z, r, ln], ysave[2 * z + 1, r, ln]))
            else:
                zs[(i0, z)] = y[i0]
            zs[(i1, z)] = fold(y[i1], y[i0])
            if p < P // 2 - 1:
                ysave[2 * z, r, ln] = y[i1][0]
                ysave[2 * z + 1, r, ln] = y[i1][1]
        for i in (i0, i1):
            (pr, pi), (qr, qi) = zs[(i, 0)], zs[(i, 1)]
            wbuf[i, 0, r, ln] = _pack(pr + qr, pi + qi)
            tok = _pack(pr - qr, pi - qi)
            wbuf[i, 1, r, ln] = tok
        chain.append(tok)
        return tok

    def INV(i, c, ph, tok=None):
        y = jnp.dot(_bf(tie(gb[pl.ds(ph * 64, 64), :], tok)), _bf(wbuf[i, ph, :, lanes(c)]),
                    preferred_element_type=f32)

        def fin():
            ybuf[i, pl.ds(ph * N2, N2), lanes(c)] = y
        return fin

    pending = []

    def flush():
        while pending:
            pending.pop(0)()

    def run_step(st, tok=None):
        fin = st(tok)
        flush()
        pending.append(fin)

    def spread(work, steps):
        n = len(steps)
        for si, st in enumerate(steps):
            lo, hi = len(work) * si // n, len(work) * (si + 1) // n
            tok = None
            for wk in work[lo:hi]:
                tok = wk()
            run_step(st, tok)

    def mac_work(p):
        return [functools.partial(MAC, p, c, rg) for c in range(NC) for rg in range(N2 // 8)]

    for j in range(P):
        cp_s[j].wait()
        cp_k[j].wait()
        cp_v[j].wait()
        if j == 0:
            cp_fh.wait()
            cp_f.wait()
            cp_shk.wait()
            zero = fb[0, 0].astype(jnp.int32) - 0x3F803F80
            holder["never"] = zero != 0
            holder["w"] = shk[...].astype(f32)
        if j % 2 == 0:
            flush()
        work = []
        if j >= 2:
            mw = mac_work(j // 2 - 1)
            work = mw[:len(mw) // 2] if j % 2 == 0 else mw[len(mw) // 2:]
        spread(work, [functools.partial(H, j, c) for c in range(NC)])
        spread([], [functools.partial(KV, j, c) for c in range(NC)])
    cp_g.wait()
    flush()
    steps = [functools.partial(INV, i, c, ph) for i in range(P - 2) for c in range(NC) for ph in range(2)]
    spread(mac_work(P // 2 - 1)[:-16], steps)
    for wk in mac_work(P // 2 - 1)[-16:]:
        wk()
    for c in range(NC):
        for i in (P - 2, P - 1):
            for ph in range(2):
                run_step(functools.partial(INV, i, c, ph))

    cp_c.wait()
    cp_dsk.wait()
    cp_wm[1].wait()
    cp_wm[0].wait()
    cp_wm[2].wait()
    flush()
    cf = cb_[...].astype(f32)
    sc = cf * (1.0 / (1.0 + jnp.exp(-cf)))
    sc = jnp.broadcast_to(sc, (16, D)).astype(bf16)

    def modpart(t):
        return jnp.dot(sc, wm[:, cols(t * D, D)], preferred_element_type=f32)[0:1]

    sa, ca, ga = modpart(0), modpart(1), modpart(2)
    ca1 = 1.0 + ca
    dskip = dsk[...].astype(f32).reshape(1, D)
    cp_q[0].wait()
    cp_wm[4].wait()
    cp_wm[3].wait()
    sb_, cb = modpart(3), modpart(4)
    cb1 = 1.0 + cb

    def ln(x):
        m = jnp.sum(x, axis=-1, keepdims=True) * (1.0 / D)
        d = x - m
        v = jnp.sum(d * d, axis=-1, keepdims=True) * (1.0 / D)
        return d * lax.rsqrt(v + EPS)

    def E(i, ph, t):
        qu = pltpu.bitcast(qb[pl.ds(i * L + 32 * t, 32), :], u32)
        xq = _lo(qu) if ph == 0 else _hi(qu)
        kvf = _bf(kvb[i, ph, pl.ds(t * 8, 8), :]).astype(f32)
        rr = pl.ds(ph * N2 + t * 16, 16)
        h = ln(xq) * ca1 + sa
        r = ybuf[i, rr, :] + kvf * dskip
        x1 = xq + ga * (h * r)
        x1b[i, rr, :] = x1
        h2 = _u(ln(x1) * cb1 + sb_)
        h2b[i, pl.ds(ph * (N2 // 2) + t * 8, 8), :] = h2
        return h2[:, D - 128:]

    def GU(i, t, tok):
        h2 = _bf(tie(h2b[i], tok))
        g = jnp.dot(h2, wg[:, lanes(t)], preferred_element_type=f32)
        u = jnp.dot(h2, wu[:, lanes(t)], preferred_element_type=f32)

        def fin():
            ab[i % 2, :, lanes(t)] = _u(g * u)
        return fin

    def DOWN(i, n, tok):
        mlp = jnp.dot(_bf(tie(ab[i % 2], tok)), wd[:, lanes(n)], preferred_element_type=f32)

        def fin():
            gbv = holder["gb"][:, lanes(n)]
            o_e = x1b[i, 0:N2, lanes(n)] + gbv * mlp[:N2]
            o_o = x1b[i, N2:L, lanes(n)] + gbv * mlp[N2:]
            ob[pl.ds(i * N2, N2), lanes(n)] = _pack(o_e, o_o)
        return fin

    pieces = [(ph, t) for t in range(N2 // 16) for ph in range(2)]
    for ph, t in pieces:
        E(0, ph, t)

    out_cps = []

    def out_copy(i0, n):
        d = cp(ob.at[pl.ds(i0 * N2, n * N2), :], o_hbm.bitcast(u32).at[pl.ds(i0 * N2, n * N2), :])
        d.start()
        out_cps.append(d)

    def gu_phase(i, e_chunk, first=False):
        e_left = [(e_chunk, ph, t) for ph, t in pieces] if e_chunk is not None else []
        tok = None
        for t in range(NF):
            if first and t % TG == 0:
                cp_wg[t // TG].wait()
                cp_wu[t // TG].wait()
                if t == TG:
                    cp_q[1].wait()
            run_step(functools.partial(GU, i, t), tok)
            tok = None
            if (not first or t >= TG) and e_left:
                per = 2 if first else (2 if t < 4 else 1)
                for _ in range(per):
                    if e_left:
                        tok = E(*e_left.pop(0))
        return e_left, tok

    def down_phase(i, e_left, tok):
        for n in range(NC):
            run_step(functools.partial(DOWN, i, n), tok)
            tok = None
            if e_left:
                tok = E(*e_left.pop(0))
        assert not e_left
        return tok

    rest, tok = gu_phase(0, 1, first=True)
    assert not rest
    flush()
    cp_q[2].wait()
    rest, tok = gu_phase(1, 2)
    cp_wd.wait()
    cp_wm[5].wait()
    holder["gb"] = modpart(5)
    flush()
    down_phase(0, rest, tok)
    flush()
    down_phase(1, [], None)
    for i in range(2, P):
        flush()
        rest, tok = gu_phase(i, i + 1 if i + 1 < P else None)
        flush()
        if i == P - 1:
            out_copy(0, P - 1)
        down_phase(i, rest, tok)
    flush()
    out_copy(P - 1, 1)
    for d in out_cps:
        d.wait()


@jax.jit
def pallas_adaLN_cond__ssm_conv_h3__glu_gated_bilinear__prompt_kernel(
    A_q, A_k, A_v, A_shift_k, A_ssm_k, A_ssm_D, B_x, B_w_gate, B_w_up, B_w_down, c, w_mod,
):
    del B_x
    f, g, fh = _dft_consts()
    hbm = pl.BlockSpec(memory_space=pl.ANY)
    out = pl.pallas_call(
        _kernel,
        in_specs=[hbm] * 14,
        out_specs=hbm,
        out_shape=jax.ShapeDtypeStruct((S, D), bf16),
        scratch_shapes=[
            pltpu.VMEM((S, D), bf16), pltpu.VMEM((S, D), bf16), pltpu.VMEM((S, D), bf16),
            pltpu.VMEM((D, S), bf16),
            pltpu.VMEM((D, F), bf16), pltpu.VMEM((D, F), bf16), pltpu.VMEM((F, D), bf16),
            pltpu.VMEM((D, 6 * D), bf16),
            pltpu.VMEM((L, N2), u32), pltpu.VMEM((N2, L), u32), pltpu.VMEM((L, L), u32),
            pltpu.VMEM((4, D), bf16), pltpu.VMEM((D,), bf16), pltpu.VMEM((1, D), bf16),
            pltpu.VMEM((P, 6, N2, D), f32),
            pltpu.VMEM((P, 6, N2, D), f32),
            pltpu.VMEM((4, N2, D), f32),
            pltpu.VMEM((P, 2, N2, D), u32),
            pltpu.VMEM((P, 2, N2 // 2, D), u32),
            pltpu.VMEM((P, L, D), f32),
            pltpu.VMEM((P, L, D), f32),
            pltpu.VMEM((P, N2, D), u32),
            pltpu.VMEM((2, N2, F), u32),
            pltpu.VMEM((S // 2, D), u32),
            pltpu.SemaphoreType.DMA((64,)),
        ],
        compiler_params=pltpu.CompilerParams(vmem_limit_bytes=120 * 1024 * 1024),
    )(A_q.reshape(S, D), A_k.reshape(S, D), A_v.reshape(S, D), A_shift_k.T, A_ssm_k,
      A_ssm_D, B_w_gate, B_w_up, B_w_down, c, w_mod, f, g, fh)
    return out.reshape(1, S, D)
```

```python
import functools

import jax
import jax.numpy as jnp
import ml_dtypes
import numpy as np
from jax import lax
import jax.experimental.pallas as pl
import jax.experimental.pallas.tpu as pltpu

CH = 1
OW = 0
S, D, F = 2048, 640, 1536
L = 256
P = S // L
N2 = L // 2
NC = D // 128
NF = F // 128
EPS = 1e-5
f32 = jnp.float32
bf16 = jnp.bfloat16
u32 = jnp.uint32


def _pack_rows(a):
    b = a.astype(ml_dtypes.bfloat16).view(np.uint16).astype(np.uint32)
    return b[0::2] | (b[1::2] << 16)


def _dft_consts():
    k = np.concatenate([np.arange(0, N2, 2), np.arange(1, N2, 2)])
    theta = (2 * k + 1) * np.pi / (2 * L)

    def mk(t):
        a = theta[:, None] * t[None, :]
        return np.cos(a), -np.sin(a)

    def mki(t):
        c, s = mk(t)
        return np.stack([c.reshape(N2 // 8, 8, -1), s.reshape(N2 // 8, 8, -1)], 1).reshape(2 * N2, -1)

    n = np.arange(N2)
    fe, fo = mki(2 * n), mki(2 * n + 1)
    t = np.arange(L)
    fp = mki(t)
    fh = np.concatenate([fp, fp * ((-1.0) ** t)[None, :]], 0)

    def mkg(t):
        c, s = mk(t)
        g = np.empty((N2, 2 * N2))
        g[:, 0::2] = c.T / L
        g[:, 1::2] = s.T / L
        return g

    g = np.concatenate([mkg(2 * n), mkg(2 * n + 1)], 0)
    return _pack_rows(np.concatenate([fe, fo], 0)), _pack_rows(g), _pack_rows(fh)


def _bf(x_u32):
    return pltpu.bitcast(x_u32, bf16)


def _u(x_f32):
    return pltpu.bitcast(x_f32.astype(bf16), u32)


def _lo(u):
    return pltpu.unpack_elementwise(u, index=0, packed_dtype=bf16, unpacked_dtype=f32)


def _hi(u):
    return pltpu.unpack_elementwise(u, index=1, packed_dtype=bf16, unpacked_dtype=f32)


def _pack(a, b):
    return pltpu.pack_elementwise([a, b], packed_dtype=bf16)


def _kernel(q_hbm, k_hbm, v_hbm, shk_hbm, ssm_hbm, dsk_hbm, wg_hbm, wu_hbm, wd_hbm,
            c_hbm, wm_hbm, f_hbm, g_hbm, fh_hbm, o_hbm,
            qb, kb, vb, sb, wg, wu, wd, wm, fb, gb, fhb, shk, dsk, cb_,
            hbuf, xbuf, ysave, wbuf, kvb, ybuf, x1b, h2b, ab, ob, n1b, sems):
    rows = lambda j: pl.ds(j * L, L)
    lanes = lambda c: slice(c * 128, (c + 1) * 128)
    nsem = [0]

    def cp(src, dst):
        nsem[0] += 1
        return pltpu.make_async_copy(src, dst, sems.at[nsem[0] - 1])

    cols = lambda a, n: pl.ds(a, n)
    cp_fh, cp_f, cp_g = cp(fh_hbm, fhb), cp(f_hbm, fb), cp(g_hbm, gb)
    cp_shk, cp_dsk, cp_c = cp(shk_hbm, shk), cp(dsk_hbm, dsk), cp(c_hbm, cb_)
    cp_s = [cp(ssm_hbm.at[:, rows(j)], sb.at[:, rows(j)]) for j in range(P)]
    cp_k = [cp(k_hbm.at[rows(j), :], kb.at[rows(j), :]) for j in range(P)]
    cp_v = [cp(v_hbm.at[rows(j), :], vb.at[rows(j), :]) for j in range(P)]
    cp_wm = [cp(wm_hbm.at[:, cols(t * D, D)], wm.at[:, cols(t * D, D)]) for t in range(6)]
    cp_q = [cp(q_hbm.at[rows(i), :], qb.at[rows(i), :]) for i in range(3)]
    cp_q.append(cp(q_hbm.at[pl.ds(3 * L, S - 3 * L), :], qb.at[pl.ds(3 * L, S - 3 * L), :]))
    TG = 3
    cp_wg = [cp(wg_hbm.at[:, cols(t * 128, TG * 128)], wg.at[0, :, cols(t * 128, TG * 128)]) for t in range(0, NF, TG)]
    cp_wu = [cp(wu_hbm.at[:, cols(t * 128, TG * 128)], wu.at[0, :, cols(t * 128, TG * 128)]) for t in range(0, NF, TG)]
    cp_wd = cp(wd_hbm, wd.at[0])

    LEAD = 1
    NA = 6
    order = [cp_fh] + cp_s[:LEAD] + [cp_f, cp_shk]
    for j in range(NA):
        order += [cp_k[j], cp_v[j]] + cp_s[j + LEAD:j + LEAD + 1]
        if j == 2:
            order += [cp_g]
    order += cp_s[NA + LEAD:]
    order += [cp_c, cp_dsk, cp_wm[1], cp_wm[0], cp_wm[2], cp_q[0], cp_wm[4], cp_wm[3], cp_q[1]]
    for t in range(NF // TG):
        order += [cp_wg[t], cp_wu[t]]
    order += [cp_q[2], cp_wd, cp_wm[5]]
    for j in range(NA, P):
        order += [cp_k[j], cp_v[j]]
    order += [cp_q[3]]
    for d in order:
        d.start()

    if 0:
        qb, kb, vb, sb, wg, wu, wd, wm, fb, gb, fhb = (
            pltpu.annotate(r, no_store=True) for r in (qb, kb, vb, sb, wg, wu, wd, wm, fb, gb, fhb))
    holder = {}

    def tie(x_u32, toks):
        if toks is None:
            return x_u32
        if not isinstance(toks, (list, tuple)):
            toks = [toks]
        toks = [t for t in toks if t is not None]
        if not toks:
            return x_u32
        ng = x_u32.shape[0] // 8
        n = len(toks)
        pos = {}
        for i, t in enumerate(toks):
            pos.setdefault((i + 1) * ng // n - 1 if n <= ng else i * ng // n, []).append(t)
        out = []
        for g in range(ng):
            blk = x_u32[8 * g:8 * g + 8]
            if g in pos:
                v = blk[:, 0:128]
                for t in pos[g]:
                    v = jnp.where(holder["never"], t, v)
                blk = v if x_u32.shape[1] == 128 else jnp.concatenate([v, blk[:, 128:]], 1)
            out.append(blk)
        return jnp.concatenate(out, 0)

    def H(m, c, tok=None):
        s = sb[lanes(c), rows(m)]
        res = []
        for z in range(2):
            fh = _bf(tie(fhb[pl.ds(z * N2, N2), :], tok if z == 0 else None))
            res.append(lax.dot_general(fh, s, (((1,), (1,)), ((), ())), preferred_element_type=f32))

        def fin():
            for z in range(2):
                for g in range(N2 // 8):
                    hr = res[z][16 * g:16 * g + 8]
                    hi = res[z][16 * g + 8:16 * g + 16]
                    hbuf[m, 3 * z + 0, pl.ds(8 * g, 8), lanes(c)] = hr
                    hbuf[m, 3 * z + 1, pl.ds(8 * g, 8), lanes(c)] = hi
                    hbuf[m, 3 * z + 2, pl.ds(8 * g, 8), lanes(c)] = hr + hi
        return fin

    sub = lax.broadcasted_iota(jnp.int32, (8, 128), 0)

    def KV(j, c, tok=None):
        w0, w1, w2, w3 = (jnp.broadcast_to(holder["w"][t:t + 1, lanes(c)], (8, 128)) for t in range(4))
        ku = pltpu.bitcast(kb[rows(j), lanes(c)], u32)
        vu = pltpu.bitcast(vb[rows(j), lanes(c)], u32)
        if j == 0:
            pe1 = po1 = po2 = jnp.zeros((8, 128), f32)
        else:
            pu = pltpu.bitcast(kb[pl.ds(j * L - 16, 16), lanes(c)], u32)
            pe, po = _lo(pu), _hi(pu)
            pe1, po1, po2 = pltpu.roll(pe, 1, 0), pltpu.roll(po, 1, 0), pltpu.roll(po, 2, 0)
        kve, kvo = [], []
        for r in range(N2 // 8):
            u = ku[r * 8:(r + 1) * 8]
            ke, ko = _lo(u), _hi(u)
            re1, ro1, ro2 = pltpu.roll(ke, 1, 0), pltpu.roll(ko, 1, 0), pltpu.roll(ko, 2, 0)
            ke1 = jnp.where(sub < 1, pe1, re1)
            ko1 = jnp.where(sub < 1, po1, ro1)
            ko2 = jnp.where(sub < 2, po2, ro2)
            pe1, po1, po2 = re1, ro1, ro2
            vv = vu[r * 8:(r + 1) * 8]
            kve.append((w0 * ke + w1 * ko1 + w2 * ke1 + w3 * ko2) * _lo(vv))
            kvo.append((w0 * ko + w1 * ke + w2 * ko1 + w3 * ke1) * _hi(vv))
        pe_ = _u(jnp.concatenate(kve, 0))
        po_ = _u(jnp.concatenate(kvo, 0))
        kvb[j, 0, :, lanes(c)] = pe_
        kvb[j, 1, :, lanes(c)] = po_
        e = jnp.dot(_bf(tie(fb[0:N2, :], tok)), _bf(pe_), preferred_element_type=f32)
        o = jnp.dot(_bf(fb[N2:L, :]), _bf(po_), preferred_element_type=f32)

        def fin():
            for g in range(N2 // 8):
                er, ei = e[16 * g:16 * g + 8], e[16 * g + 8:16 * g + 16]
                or_, oi = o[16 * g:16 * g + 8], o[16 * g + 8:16 * g + 16]
                for z, (xr, xi) in enumerate(((er + or_, ei + oi), (er - or_, ei - oi))):
                    xbuf[j, 3 * z + 0, pl.ds(8 * g, 8), lanes(c)] = xr
                    xbuf[j, 3 * z + 1, pl.ds(8 * g, 8), lanes(c)] = xi
                    xbuf[j, 3 * z + 2, pl.ds(8 * g, 8), lanes(c)] = xr + xi
        fin.tok = pltpu.bitcast(e[0 * 8:0 * 8 + 8], u32)
        return fin

    chain = []

    def MAC(p, c, rg):
        i0, i1 = 2 * p, 2 * p + 1
        r = pl.ds(rg * 8, 8)
        ln = lanes(c)
        even = rg < N2 // 16
        zs = {}
        for z in range(2):
            acc = {}
            xs_ = {}

            def X(j):
                if j not in xs_:
                    xs_[j] = tuple(xbuf[j, 3 * z + t, r, ln] for t in range(3))
                return xs_[j]

            for m in range(i1 + 1):
                hh = tuple(hbuf[m, 3 * z + t, r, ln] for t in range(3))
                if m == 0 and z == 0 and len(chain) >= CH and CH > 0:
                    hh = (jnp.where(holder["never"], pltpu.bitcast(chain[-CH], f32), hh[0]),) + hh[1:]
                for i in (i1, i0):
                    j = i - m
                    if j < 0:
                        continue
                    xx = X(j)
                    t3 = tuple(a * b for a, b in zip(hh, xx))
                    acc[i] = t3 if i not in acc else tuple(a + b for a, b in zip(acc[i], t3))
            y = {}
            for i in (i0, i1):
                a, b, cc = acc[i]
                y[i] = (a - b, cc - a - b)

            def fold(yy, pv):
                if even:
                    return yy[0] - pv[1], yy[1] + pv[0]
                return yy[0] + pv[1], yy[1] - pv[0]

            if p > 0:
                zs[(i0, z)] = fold(y[i0], (ysave[2 * z, r, ln], ysave[2 * z + 1, r, ln]))
            else:
                zs[(i0, z)] = y[i0]
            zs[(i1, z)] = fold(y[i1], y[i0])
            if p < P // 2 - 1:
                ysave[2 * z, r, ln] = y[i1][0]
                ysave[2 * z + 1, r, ln] = y[i1][1]
        for i in (i0, i1):
            (pr, pi), (qr, qi) = zs[(i, 0)], zs[(i, 1)]
            wbuf[i, 0, r, ln] = _pack(pr + qr, pi + qi)
            tok = _pack(pr - qr, pi - qi)
            wbuf[i, 1, r, ln] = tok
        chain.append(tok)
        return tok

    def INV(i, c, ph, tok=None):
        y = jnp.dot(_bf(tie(gb[pl.ds(ph * 64, 64), :], tok)), _bf(wbuf[i, ph, :, lanes(c)]),
                    preferred_element_type=f32)

        def fin():
            ybuf[i, pl.ds(ph * N2, N2), lanes(c)] = y
        return fin

    pending = []

    def flush():
        while pending:
            pending.pop(0)()

    def run_step(st, tok=None):
        fin = st(tok)
        flush()
        pending.append(fin)
        return fin

    def spread(work, steps):
        n = len(steps)
        for si, st in enumerate(steps):
            lo, hi = len(work) * si // n, len(work) * (si + 1) // n
            run_step(st, [wk() for wk in work[lo:hi]])

    def mac_work(p):
        return [functools.partial(MAC, p, c, rg) for c in range(NC) for rg in range(N2 // 8)]

    hs = lambda m: [functools.partial(H, m, c) for c in range(NC)]
    xs = lambda j: [functools.partial(KV, j, c) for c in range(NC)]
    invs = lambda i: [functools.partial(INV, i, c, ph) for c in range(NC) for ph in range(2)]
    for m in range(LEAD):
        cp_s[m].wait()
        if m == 0:
            cp_fh.wait()
        spread([], hs(m))
    for j in range(P):
        if j < NA:
            cp_k[j].wait()
            cp_v[j].wait()
        if j + LEAD < P:
            cp_s[j + LEAD].wait()
        if j == 0:
            if LEAD == 0:
                cp_fh.wait()
            cp_f.wait()
            cp_shk.wait()
            zero = fb[0, 0].astype(jnp.int32) - 0x3F803F80
            holder["never"] = zero != 0
            holder["zero"] = zero
            holder["w"] = shk[...].astype(f32)
        if j == 4:
            cp_g.wait()
        if j % 2 == 0:
            flush()
        work = []
        if j >= 2:
            mw = mac_work(j // 2 - 1)
            work = mw[:len(mw) // 2] if j % 2 == 0 else mw[len(mw) // 2:]
        st_h = hs(j + LEAD) if j + LEAD < P else []
        st_x = xs(j) if j < NA else []
        st_i = invs(j - 4) if j >= 4 else []
        if st_h:
            spread(work, st_h)
            rest = []
            for c in range(NC):
                rest += st_x[c:c + 1] + st_i[2 * c:2 * c + 2]
            spread([], rest)
        else:
            rest = []
            for c in range(NC):
                rest += st_x[c:c + 1] + st_i[2 * c:2 * c + 2]
            spread(work, rest)
    flush()
    for c in range(NC):
        for i in (P - 4, P - 3):
            for ph in range(2):
                run_step(functools.partial(INV, i, c, ph))

    cp_c.wait()
    cp_dsk.wait()
    cp_wm[1].wait()
    cp_wm[0].wait()
    cp_wm[2].wait()
    flush()
    cf = cb_[...].astype(f32)
    sc = cf * (1.0 / (1.0 + jnp.exp(-cf)))
    sc = jnp.broadcast_to(sc, (16, D)).astype(bf16)

    def modpart(t):
        return jnp.dot(sc, wm[:, cols(t * D, D)], preferred_element_type=f32)[0:1]

    sa, ca, ga = modpart(0), modpart(1), modpart(2)
    ca1 = 1.0 + ca
    dskip = dsk[...].astype(f32).reshape(1, D)

    def ln(x):
        m = jnp.sum(x, axis=-1, keepdims=True) * (1.0 / D)
        d = x - m
        v = jnp.sum(d * d, axis=-1, keepdims=True) * (1.0 / D)
        return d * lax.rsqrt(v + EPS)

    def Ea(i, ph, t):
        qu = pltpu.bitcast(qb[pl.ds(i * L + 32 * t, 32), :], u32)
        xq = _lo(qu) if ph == 0 else _hi(qu)
        kvf = _bf(kvb[i, ph, pl.ds(t * 8, 8), :]).astype(f32)
        rr = pl.ds(ph * N2 + t * 16, 16)
        h = ln(xq) * ca1 + sa
        r = ybuf[i, rr, :] + kvf * dskip
        x1 = xq + ga * (h * r)
        x1b[i, rr, :] = x1
        return ln(x1)

    def Eb(i, ph, t, n1):
        h2 = _u(n1 * holder["cb1"] + holder["sb"])
        h2b[i, pl.ds(ph * (N2 // 2) + t * 8, 8), :] = h2
        return h2[:, D - 128:]

    def E(i, ph, t):
        return Eb(i, ph, t, Ea(i, ph, t))

    def GU(i, t, tok):
        h2 = _bf(tie(h2b[i], tok))
        zi = holder["zero"] * (i + 1) if OW else 0
        g = jnp.dot(h2, wg[zi, :, lanes(t)], preferred_element_type=f32)
        u = jnp.dot(h2, wu[zi, :, lanes(t)], preferred_element_type=f32)

        def fin():
            ab[i % 2, :, lanes(t)] = _u(g * u)
        return fin

    def DOWN(i, n, tok):
        zi = holder["zero"] * (i + 1) if OW else 0
        mlp = jnp.dot(_bf(tie(ab[i % 2], tok)), wd[zi, :, lanes(n)], preferred_element_type=f32)

        def fin():
            gbv = holder["gb"][:, lanes(n)]
            o_e = x1b[i, 0:N2, lanes(n)] + gbv * mlp[:N2]
            o_o = x1b[i, N2:L, lanes(n)] + gbv * mlp[N2:]
            ob[pl.ds(i * N2, N2), lanes(n)] = _pack(o_e, o_o)
        return fin

    pieces = [(ph, t) for t in range(N2 // 16) for ph in range(2)]
    cp_q[0].wait()
    for ph, t in pieces:
        n1b[pl.ds(ph * N2 + t * 16, 16), :] = Ea(0, ph, t)
    cp_wm[4].wait()
    cp_wm[3].wait()
    holder["sb"] = modpart(3)
    holder["cb1"] = 1.0 + modpart(4)
    for ph, t in pieces:
        Eb(0, ph, t, n1b[pl.ds(ph * N2 + t * 16, 16), :])

    out_cps = []

    def out_copy(i0, n):
        d = cp(ob.at[pl.ds(i0 * N2, n * N2), :], o_hbm.bitcast(u32).at[pl.ds(i0 * N2, n * N2), :])
        d.start()
        out_cps.append(d)

    def phase(steps, work):
        n = len(steps)
        tok = carry[0]
        for si, st in enumerate(steps):
            lo, hi = len(work) * si // n, len(work) * (si + 1) // n
            run_step(st, tok)
            tok = [wk() for wk in work[lo:hi]]
        carry[0] = tok

    carry = [None]
    ew = lambda i: [functools.partial(E, i, ph, t) for ph, t in pieces]
    gu = lambda i: [functools.partial(GU, i, t) for t in range(NF)]
    dn = lambda i: [functools.partial(DOWN, i, n) for n in range(NC)]

    def mix(a, b):
        out = [(float(i + 0.5) / len(a), 0, w_) for i, w_ in enumerate(a)] + [(float(i + 0.5) / len(b), 1, w_) for i, w_ in enumerate(b)]
        return [w_ for _, _, w_ in sorted(out, key=lambda x: (x[0], x[1]))]

    def fence():
        return ob[pl.ds(pl.multiple_of(jnp.clip(holder["zero"], 0, S // 2 - 8), 8), 8), 0:128]
    e1, e2 = ew(1), ew(2)
    NG = NF // TG
    for tg in range(NG):
        cp_wg[tg].wait()
        cp_wu[tg].wait()
        if tg == 0:
            cp_q[1].wait()
            phase(gu(0)[:TG], e1)
            flush()
            phase(gu(1)[:TG], [])
        else:
            if tg == NG - 1:
                cp_q[2].wait()
            phase(gu(0)[tg * TG:(tg + 1) * TG] + gu(1)[tg * TG:(tg + 1) * TG],
                  e2 if tg == NG - 1 else [])
    late = mac_work(P // 2 - 1)
    cp_wd.wait()
    cp_wm[5].wait()
    for j in range(NA, P):
        cp_k[j].wait()
        cp_v[j].wait()
    holder["gb"] = modpart(5)
    flush()
    lx = [s_ for j in range(NA, P) for s_ in xs(j)]
    phase(mix(dn(0) + dn(1), lx) if lx else dn(0) + dn(1), [])
    n3 = len(late)
    LS = [int(x) for x in "35,70".split(",")]
    share = {2: late[:n3 * LS[0] // 100], 3: late[n3 * LS[0] // 100:n3 * LS[1] // 100], 4: late[n3 * LS[1] // 100:]}
    for i in range(2, P):
        flush()
        if i == 2:
            cp_q[3].wait()
        work = ew(i + 1) if i + 1 < P else []
        lw = share.get(i, [])
        steps = gu(i)
        nw = len(lw) * NF // (NF + NC) if i < 4 else len(lw)
        wk = mix(work[:NF], lw[:nw]) if lw else work[:NF]
        if i == P - 1:
            phase(steps[:4], [])
            out_copy(0, P - 1)
            phase(steps[4:], [])
        else:
            phase(steps, wk)
        flush()
        dsteps = dn(i) if i != 4 else mix(dn(i), invs(P - 2) + invs(P - 1))
        phase(dsteps, mix(work[NF:], lw[nw:]) if lw[nw:] else work[NF:])
    flush()
    out_copy(P - 1, 1)
    for d in out_cps:
        d.wait()


@jax.jit
def pallas_adaLN_cond__ssm_conv_h3__glu_gated_bilinear__prompt_kernel(
    A_q, A_k, A_v, A_shift_k, A_ssm_k, A_ssm_D, B_x, B_w_gate, B_w_up, B_w_down, c, w_mod,
):
    del B_x
    f, g, fh = _dft_consts()
    hbm = pl.BlockSpec(memory_space=pl.ANY)
    out = pl.pallas_call(
        _kernel,
        in_specs=[hbm] * 14,
        out_specs=hbm,
        out_shape=jax.ShapeDtypeStruct((S, D), bf16),
        scratch_shapes=[
            pltpu.VMEM((S, D), bf16), pltpu.VMEM((S, D), bf16), pltpu.VMEM((S, D), bf16),
            pltpu.VMEM((D, S), bf16),
            pltpu.VMEM((1, D, F), bf16), pltpu.VMEM((1, D, F), bf16), pltpu.VMEM((1, F, D), bf16),
            pltpu.VMEM((D, 6 * D), bf16),
            pltpu.VMEM((L, N2), u32), pltpu.VMEM((N2, L), u32), pltpu.VMEM((L, L), u32),
            pltpu.VMEM((4, D), bf16), pltpu.VMEM((D,), bf16), pltpu.VMEM((1, D), bf16),
            pltpu.VMEM((P, 6, N2, D), f32),
            pltpu.VMEM((P, 6, N2, D), f32),
            pltpu.VMEM((4, N2, D), f32),
            pltpu.VMEM((P, 2, N2, D), u32),
            pltpu.VMEM((P, 2, N2 // 2, D), u32),
            pltpu.VMEM((P, L, D), f32),
            pltpu.VMEM((P, L, D), f32),
            pltpu.VMEM((P, N2, D), u32),
            pltpu.VMEM((2, N2, F), u32),
            pltpu.VMEM((S // 2, D), u32),
            pltpu.VMEM((L, D), f32),
            pltpu.SemaphoreType.DMA((64,)),
        ],
        compiler_params=pltpu.CompilerParams(vmem_limit_bytes=120 * 1024 * 1024),
    )(A_q.reshape(S, D), A_k.reshape(S, D), A_v.reshape(S, D), A_shift_k.T, A_ssm_k,
      A_ssm_D, B_w_gate, B_w_up, B_w_down, c, w_mod, f, g, fh)
    return out.reshape(1, S, D)
```

```python
import functools

import jax
import jax.numpy as jnp

import numpy as np
from jax import lax
import jax.experimental.pallas as pl
import jax.experimental.pallas.tpu as pltpu

CH = 1
OW = 0
S, D, F = 2048, 640, 1536
L = 256
P = S // L
N2 = L // 2
NC = D // 128
NF = F // 128
EPS = 1e-5
f32 = jnp.float32
bf16 = jnp.bfloat16
u32 = jnp.uint32


def _bf(x_u32):
    return pltpu.bitcast(x_u32, bf16)


def _u(x_f32):
    return pltpu.bitcast(x_f32.astype(bf16), u32)


def _lo(u):
    return pltpu.unpack_elementwise(u, index=0, packed_dtype=bf16, unpacked_dtype=f32)


def _hi(u):
    return pltpu.unpack_elementwise(u, index=1, packed_dtype=bf16, unpacked_dtype=f32)


def _pack(a, b):
    return pltpu.pack_elementwise([a, b], packed_dtype=bf16)


def _kernel(q_hbm, k_hbm, v_hbm, shk_hbm, ssm_hbm, dsk_hbm, wg_hbm, wu_hbm, wd_hbm,
            c_hbm, wm_hbm, o_hbm,
            qb, kb, vb, sb, wg, wu, wd, wm, fb, gb, fhb, shk, dsk, cb_,
            hbuf, xbuf, ysave, wbuf, kvb, ybuf, x1b, h2b, ab, ob, n1b, sems):
    rows = lambda j: pl.ds(j * L, L)
    lanes = lambda c: slice(c * 128, (c + 1) * 128)
    nsem = [0]

    def cp(src, dst):
        nsem[0] += 1
        return pltpu.make_async_copy(src, dst, sems.at[nsem[0] - 1])

    cols = lambda a, n: pl.ds(a, n)
    cp_shk, cp_dsk, cp_c = cp(shk_hbm, shk), cp(dsk_hbm, dsk), cp(c_hbm, cb_)
    cp_s = [cp(ssm_hbm.at[:, rows(j)], sb.at[:, rows(j)]) for j in range(P)]
    cp_k = [cp(k_hbm.at[rows(j), :], kb.at[rows(j), :]) for j in range(P)]
    cp_v = [cp(v_hbm.at[rows(j), :], vb.at[rows(j), :]) for j in range(P)]
    cp_wm = [cp(wm_hbm.at[:, cols(t * D, D)], wm.at[:, cols(t * D, D)]) for t in range(6)]
    cp_q = [cp(q_hbm.at[rows(i), :], qb.at[rows(i), :]) for i in range(3)]
    cp_q.append(cp(q_hbm.at[pl.ds(3 * L, S - 3 * L), :], qb.at[pl.ds(3 * L, S - 3 * L), :]))
    TG = 3
    cp_wg = [cp(wg_hbm.at[:, cols(t * 128, TG * 128)], wg.at[0, :, cols(t * 128, TG * 128)]) for t in range(0, NF, TG)]
    cp_wu = [cp(wu_hbm.at[:, cols(t * 128, TG * 128)], wu.at[0, :, cols(t * 128, TG * 128)]) for t in range(0, NF, TG)]
    cp_wd = cp(wd_hbm, wd.at[0])

    LEAD = 0
    NA = 6
    order = cp_s[:LEAD] + [cp_shk]
    for j in range(NA):
        order += [cp_k[j], cp_v[j]] + cp_s[j + LEAD:j + LEAD + 1]
    order += cp_s[NA + LEAD:]
    order += [cp_c, cp_dsk, cp_wm[1], cp_wm[0], cp_wm[2], cp_q[0], cp_wm[4], cp_wm[3], cp_q[1]]
    for t in range(NF // TG):
        order += [cp_wg[t], cp_wu[t]]
    order += [cp_q[2], cp_wd, cp_wm[5]]
    for j in range(NA, P):
        order += [cp_k[j], cp_v[j]]
    order += [cp_q[3]]
    STOP = 0
    if STOP == 1:
        order = order[:[id(o) for o in order].index(id(cp_q[1]))]
    if STOP == 2:
        order = order[:[id(o) for o in order].index(id(cp_wd))]
    for d in order:
        d.start()

    if 0:
        qb, kb, vb, sb, wg, wu, wd, wm, fb, gb, fhb = (
            pltpu.annotate(r, no_store=True) for r in (qb, kb, vb, sb, wg, wu, wd, wm, fb, gb, fhb))
    s8 = lax.broadcasted_iota(jnp.int32, (8, 128), 0)
    l8 = lax.broadcasted_iota(jnp.int32, (8, 128), 1)

    def cis(idx):
        ang = (idx & (4 * L - 1)).astype(f32) * np.float32(np.pi / (2 * L))
        return jnp.cos(ang), -jnp.sin(ang)

    def walk(z, rot, n):
        out = [z]
        for _ in range(n - 1):
            z = (z[0] * rot[0] - z[1] * rot[1], z[0] * rot[1] + z[1] * rot[0])
            out.append(z)
        return out

    def fwd_rows(t):
        rot = cis(32 * t)
        zs = walk(cis((4 * s8 + 1) * t), rot, 8) + walk(cis((4 * s8 + 3) * t), rot, 8)
        return jnp.concatenate([p for z in zs for p in z], 0)

    for ct in range(2):
        t = l8 + 128 * ct
        fp = fwd_rows(t)
        fhb[0:N2, lanes(ct)] = _u(fp)
        fhb[N2:L, lanes(ct)] = _u(jnp.where((t[0:1] & 1) == 1, -fp, fp))
    for ph in range(2):
        fb[pl.ds(ph * N2, N2), :] = _u(fwd_rows(2 * l8 + ph))
        for ct in range(2):
            kk = 2 * (l8 >> 1) + ct
            zs = walk(cis((2 * kk + 1) * (2 * s8 + ph)), cis((2 * kk + 1) * 16), 16)
            g = jnp.concatenate([jnp.where((l8 & 1) == 0, z[0], z[1]) for z in zs], 0)
            gb[pl.ds(ph * 64, 64), lanes(ct)] = _u(g * np.float32(1.0 / L))

    holder = {}

    def tie(x_u32, toks):
        if toks is None:
            return x_u32
        if not isinstance(toks, (list, tuple)):
            toks = [toks]
        toks = [t for t in toks if t is not None]
        if not toks:
            return x_u32
        ng = x_u32.shape[0] // 8
        n = len(toks)
        pos = {}
        for i, t in enumerate(toks):
            pos.setdefault((i + 1) * ng // n - 1 if n <= ng else i * ng // n, []).append(t)
        out = []
        for g in range(ng):
            blk = x_u32[8 * g:8 * g + 8]
            if g in pos:
                v = blk[:, 0:128]
                for t in pos[g]:
                    v = jnp.where(holder["never"], t, v)
                blk = v if x_u32.shape[1] == 128 else jnp.concatenate([v, blk[:, 128:]], 1)
            out.append(blk)
        return jnp.concatenate(out, 0)

    def H(m, c, tok=None):
        s = sb[lanes(c), rows(m)]
        res = []
        for z in range(2):
            fh = _bf(tie(fhb[pl.ds(z * N2, N2), :], tok if z == 0 else None))
            res.append(lax.dot_general(fh, s, (((1,), (1,)), ((), ())), preferred_element_type=f32))

        def fin():
            for z in range(2):
                for g in range(N2 // 8):
                    hr = res[z][16 * g:16 * g + 8]
                    hi = res[z][16 * g + 8:16 * g + 16]
                    hbuf[m, 3 * z + 0, pl.ds(8 * g, 8), lanes(c)] = hr
                    hbuf[m, 3 * z + 1, pl.ds(8 * g, 8), lanes(c)] = hi
                    hbuf[m, 3 * z + 2, pl.ds(8 * g, 8), lanes(c)] = hr + hi
        return fin

    sub = lax.broadcasted_iota(jnp.int32, (8, 128), 0)

    def KV(j, c, tok=None):
        w0, w1, w2, w3 = (jnp.broadcast_to(holder["w"][t:t + 1, lanes(c)], (8, 128)) for t in range(4))
        ku = pltpu.bitcast(kb[rows(j), lanes(c)], u32)
        vu = pltpu.bitcast(vb[rows(j), lanes(c)], u32)
        if j == 0:
            pe1 = po1 = po2 = jnp.zeros((8, 128), f32)
        else:
            pu = pltpu.bitcast(kb[pl.ds(j * L - 16, 16), lanes(c)], u32)
            pe, po = _lo(pu), _hi(pu)
            pe1, po1, po2 = pltpu.roll(pe, 1, 0), pltpu.roll(po, 1, 0), pltpu.roll(po, 2, 0)
        kve, kvo = [], []
        for r in range(N2 // 8):
            u = ku[r * 8:(r + 1) * 8]
            ke, ko = _lo(u), _hi(u)
            re1, ro1, ro2 = pltpu.roll(ke, 1, 0), pltpu.roll(ko, 1, 0), pltpu.roll(ko, 2, 0)
            ke1 = jnp.where(sub < 1, pe1, re1)
            ko1 = jnp.where(sub < 1, po1, ro1)
            ko2 = jnp.where(sub < 2, po2, ro2)
            pe1, po1, po2 = re1, ro1, ro2
            vv = vu[r * 8:(r + 1) * 8]
            kve.append((w0 * ke + w1 * ko1 + w2 * ke1 + w3 * ko2) * _lo(vv))
            kvo.append((w0 * ko + w1 * ke + w2 * ko1 + w3 * ke1) * _hi(vv))
        pe_ = _u(jnp.concatenate(kve, 0))
        po_ = _u(jnp.concatenate(kvo, 0))
        kvb[j, 0, :, lanes(c)] = pe_
        kvb[j, 1, :, lanes(c)] = po_
        e = jnp.dot(_bf(tie(fb[0:N2, :], tok)), _bf(pe_), preferred_element_type=f32)
        o = jnp.dot(_bf(fb[N2:L, :]), _bf(po_), preferred_element_type=f32)

        def fin():
            for g in range(N2 // 8):
                er, ei = e[16 * g:16 * g + 8], e[16 * g + 8:16 * g + 16]
                or_, oi = o[16 * g:16 * g + 8], o[16 * g + 8:16 * g + 16]
                for z, (xr, xi) in enumerate(((er + or_, ei + oi), (er - or_, ei - oi))):
                    xbuf[j, 3 * z + 0, pl.ds(8 * g, 8), lanes(c)] = xr
                    xbuf[j, 3 * z + 1, pl.ds(8 * g, 8), lanes(c)] = xi
                    xbuf[j, 3 * z + 2, pl.ds(8 * g, 8), lanes(c)] = xr + xi
        fin.tok = pltpu.bitcast(e[0 * 8:0 * 8 + 8], u32)
        return fin

    chain = []

    def MAC(p, c, rg):
        i0, i1 = 2 * p, 2 * p + 1
        r = pl.ds(rg * 8, 8)
        ln = lanes(c)
        even = rg < N2 // 16
        zs = {}
        for z in range(2):
            acc = {}
            xs_ = {}

            def X(j):
                if j not in xs_:
                    xs_[j] = tuple(xbuf[j, 3 * z + t, r, ln] for t in range(3))
                return xs_[j]

            for m in range(i1 + 1):
                hh = tuple(hbuf[m, 3 * z + t, r, ln] for t in range(3))
                if m == 0 and z == 0 and len(chain) >= CH and CH > 0:
                    hh = (jnp.where(holder["never"], pltpu.bitcast(chain[-CH], f32), hh[0]),) + hh[1:]
                for i in (i1, i0):
                    j = i - m
                    if j < 0:
                        continue
                    xx = X(j)
                    t3 = tuple(a * b for a, b in zip(hh, xx))
                    acc[i] = t3 if i not in acc else tuple(a + b for a, b in zip(acc[i], t3))
            y = {}
            for i in (i0, i1):
                a, b, cc = acc[i]
                y[i] = (a - b, cc - a - b)

            def fold(yy, pv):
                if even:
                    return yy[0] - pv[1], yy[1] + pv[0]
                return yy[0] + pv[1], yy[1] - pv[0]

            if p > 0:
                zs[(i0, z)] = fold(y[i0], (ysave[2 * z, r, ln], ysave[2 * z + 1, r, ln]))
            else:
                zs[(i0, z)] = y[i0]
            zs[(i1, z)] = fold(y[i1], y[i0])
            if p < P // 2 - 1:
                ysave[2 * z, r, ln] = y[i1][0]
                ysave[2 * z + 1, r, ln] = y[i1][1]
        for i in (i0, i1):
            (pr, pi), (qr, qi) = zs[(i, 0)], zs[(i, 1)]
            wbuf[i, 0, r, ln] = _pack(pr + qr, pi + qi)
            tok = _pack(pr - qr, pi - qi)
            wbuf[i, 1, r, ln] = tok
        chain.append(tok)
        return tok

    def INV(i, c, ph, tok=None):
        y = jnp.dot(_bf(tie(gb[pl.ds(ph * 64, 64), :], tok)), _bf(wbuf[i, ph, :, lanes(c)]),
                    preferred_element_type=f32)

        def fin():
            ybuf[i, pl.ds(ph * N2, N2), lanes(c)] = y
        return fin

    pending = []

    def flush():
        while pending:
            pending.pop(0)()

    def run_step(st, tok=None):
        fin = st(tok)
        flush()
        pending.append(fin)
        return fin

    def spread(work, steps):
        n = len(steps)
        for si, st in enumerate(steps):
            lo, hi = len(work) * si // n, len(work) * (si + 1) // n
            run_step(st, [wk() for wk in work[lo:hi]])

    def mac_work(p):
        return [functools.partial(MAC, p, c, rg) for c in range(NC) for rg in range(N2 // 8)]

    def modpart(t):
        return jnp.dot(holder["sc"], wm[:, cols(t * D, D)], preferred_element_type=f32)[0:1]

    hs = lambda m: [functools.partial(H, m, c) for c in range(NC)]
    xs = lambda j: [functools.partial(KV, j, c) for c in range(NC)]
    invs = lambda i: [functools.partial(INV, i, c, ph) for c in range(NC) for ph in range(2)]
    for m in range(LEAD):
        cp_s[m].wait()
        spread([], hs(m))
    for j in range(P):
        if j < NA:
            cp_k[j].wait()
            cp_v[j].wait()
        if j + LEAD < P:
            cp_s[j + LEAD].wait()
        if j == 0:
            cp_shk.wait()
            zero = fb[0, 0].astype(jnp.int32) - 0x3F803F80
            holder["never"] = zero != 0
            holder["zero"] = zero
            holder["w"] = shk[...].astype(f32)
        if j == P - 1:
            cp_c.wait()
            cp_dsk.wait()
            cp_wm[1].wait()
            cp_wm[0].wait()
            cp_wm[2].wait()
            cp_q[0].wait()
            cf = cb_[...].astype(f32)
            sc = cf * (1.0 / (1.0 + jnp.exp(-cf)))
            holder["sc"] = jnp.broadcast_to(sc, (16, D)).astype(bf16)
            sa, ca, ga = modpart(0), modpart(1), modpart(2)
            ca1 = 1.0 + ca
            dskip = dsk[...].astype(f32).reshape(1, D)
        if j % 2 == 0:
            flush()
        work = []
        if j >= 2:
            mw = mac_work(j // 2 - 1)
            work = mw[:len(mw) // 2] if j % 2 == 0 else mw[len(mw) // 2:]
        st_h = hs(j + LEAD) if j + LEAD < P else []
        st_x = xs(j) if j < NA else []
        st_i = invs(j - 4) if j >= 4 else []
        if st_h:
            spread(work, st_h)
            rest = []
            for c in range(NC):
                rest += st_x[c:c + 1] + st_i[2 * c:2 * c + 2]
            spread([], rest)
        else:
            rest = []
            for c in range(NC):
                rest += st_x[c:c + 1] + st_i[2 * c:2 * c + 2]
            spread(work, rest)
    def ln(x):
        m = jnp.sum(x, axis=-1, keepdims=True) * (1.0 / D)
        d = x - m
        v = jnp.sum(d * d, axis=-1, keepdims=True) * (1.0 / D)
        return d * lax.rsqrt(v + EPS)

    def Ea(i, ph, t):
        qu = pltpu.bitcast(qb[pl.ds(i * L + 32 * t, 32), :], u32)
        xq = _lo(qu) if ph == 0 else _hi(qu)
        kvf = _bf(kvb[i, ph, pl.ds(t * 8, 8), :]).astype(f32)
        rr = pl.ds(ph * N2 + t * 16, 16)
        h = ln(xq) * ca1 + sa
        r = ybuf[i, rr, :] + kvf * dskip
        x1 = xq + ga * (h * r)
        x1b[i, rr, :] = x1
        return ln(x1)

    def Eb(i, ph, t, n1):
        h2 = _u(n1 * holder["cb1"] + holder["sb"])
        h2b[i, pl.ds(ph * (N2 // 2) + t * 8, 8), :] = h2
        return h2[:, D - 128:]

    def E(i, ph, t):
        return Eb(i, ph, t, Ea(i, ph, t))

    def GU(i, t, tok):
        h2 = _bf(tie(h2b[i], tok))
        zi = holder["zero"] * (i + 1) if OW else 0
        g = jnp.dot(h2, wg[zi, :, lanes(t)], preferred_element_type=f32)
        u = jnp.dot(h2, wu[zi, :, lanes(t)], preferred_element_type=f32)

        def fin():
            ab[i % 2, :, lanes(t)] = _u(g * u)
        return fin

    def DOWN(i, n, tok):
        zi = holder["zero"] * (i + 1) if OW else 0
        mlp = jnp.dot(_bf(tie(ab[i % 2], tok)), wd[zi, :, lanes(n)], preferred_element_type=f32)

        def fin():
            gbv = holder["gb"][:, lanes(n)]
            o_e = x1b[i, 0:N2, lanes(n)] + gbv * mlp[:N2]
            o_o = x1b[i, N2:L, lanes(n)] + gbv * mlp[N2:]
            ob[pl.ds(i * N2, N2), lanes(n)] = _pack(o_e, o_o)
        return fin

    pieces = [(ph, t) for t in range(N2 // 16) for ph in range(2)]
    def Ea0(ph, t):
        n1 = Ea(0, ph, t)
        n1b[pl.ds(ph * N2 + t * 16, 16), :] = n1
        return pltpu.bitcast(n1[0:8, D - 128:], u32)

    tail_steps = [functools.partial(INV, i, c, ph) for c in range(NC) for i in (P - 4, P - 3) for ph in range(2)]
    spread([functools.partial(Ea0, ph, t) for ph, t in pieces], tail_steps)
    cp_wm[4].wait()
    cp_wm[3].wait()
    flush()
    holder["sb"] = modpart(3)
    holder["cb1"] = 1.0 + modpart(4)
    for ph, t in pieces:
        Eb(0, ph, t, n1b[pl.ds(ph * N2 + t * 16, 16), :])

    out_cps = []
    if STOP == 1:
        ob[0:N2, :] = h2b[0]
        d = cp(ob.at[pl.ds(0, N2), :], o_hbm.bitcast(u32).at[pl.ds(0, N2), :])
        d.start()
        d.wait()
        return

    def out_copy(i0, n):
        d = cp(ob.at[pl.ds(i0 * N2, n * N2), :], o_hbm.bitcast(u32).at[pl.ds(i0 * N2, n * N2), :])
        d.start()
        out_cps.append(d)

    def phase(steps, work):
        n = len(steps)
        tok = carry[0]
        for si, st in enumerate(steps):
            lo, hi = len(work) * si // n, len(work) * (si + 1) // n
            run_step(st, tok)
            tok = [wk() for wk in work[lo:hi]]
        carry[0] = tok

    carry = [None]
    ew = lambda i: [functools.partial(E, i, ph, t) for ph, t in pieces]
    gu = lambda i: [functools.partial(GU, i, t) for t in range(NF)]
    dn = lambda i: [functools.partial(DOWN, i, n) for n in range(NC)]

    def mix(a, b):
        out = [(float(i + 0.5) / len(a), 0, w_) for i, w_ in enumerate(a)] + [(float(i + 0.5) / len(b), 1, w_) for i, w_ in enumerate(b)]
        return [w_ for _, _, w_ in sorted(out, key=lambda x: (x[0], x[1]))]

    def fence():
        return ob[pl.ds(pl.multiple_of(jnp.clip(holder["zero"], 0, S // 2 - 8), 8), 8), 0:128]
    e1, e2 = ew(1), ew(2)
    NG = NF // TG
    GW = [int(x) for x in "0,1,2,3".split(",")]
    E1N = 3
    for tg in range(NG):
        for t in range(NG):
            if GW[t] == tg:
                cp_wg[t].wait()
                cp_wu[t].wait()
        if tg == 0:
            cp_q[1].wait()
            phase(gu(0)[:E1N], e1)
            phase(gu(0)[E1N:TG], [])
            flush()
            phase(gu(1)[:TG], [])
        else:
            if tg == max(GW):
                cp_q[2].wait()
            phase(gu(0)[tg * TG:(tg + 1) * TG] + gu(1)[tg * TG:(tg + 1) * TG],
                  e2 if tg == NG - 1 else [])
    if STOP == 2:
        flush()
        ob[0:N2, :] = h2b[2]
        ob[N2:2 * N2, :] = ab[1][:, 0:D]
        d = cp(ob.at[pl.ds(0, 2 * N2), :], o_hbm.bitcast(u32).at[pl.ds(0, 2 * N2), :])
        d.start()
        d.wait()
        return
    late = mac_work(P // 2 - 1)
    if 0:
        late = late[:5]
    cp_wd.wait()
    cp_wm[5].wait()
    XL = 0
    if not XL:
        for j in range(NA, P):
            cp_k[j].wait()
            cp_v[j].wait()
    holder["gb"] = modpart(5)
    flush()
    lx = [s_ for j in range(NA, P) for s_ in xs(j)]
    phase(mix(dn(0) + dn(1), lx) if lx and not XL else dn(0) + dn(1), [])
    def stop_here(n):
        flush()
        d = cp(ob.at[pl.ds(0, n * N2), :], o_hbm.bitcast(u32).at[pl.ds(0, n * N2), :])
        d.start()
        d.wait()
        if STOP == 3:
            cp_q[3].wait()
    if STOP == 3:
        stop_here(1)
        return
    n3 = len(late)
    LS = [int(x) for x in "35,70".split(",")]
    share = {2: late[:n3 * LS[0] // 100], 3: late[n3 * LS[0] // 100:n3 * LS[1] // 100], 4: late[n3 * LS[1] // 100:]}
    for i in range(2, P):
        flush()
        if i == 2:
            cp_q[3].wait()
            if XL:
                for j in range(NA, P):
                    cp_k[j].wait()
                    cp_v[j].wait()
        work = ew(i + 1) if i + 1 < P else []
        if 0 and i + 1 < P:
            work = work[:2]
        lw = share.get(i, [])
        steps = gu(i)
        if XL and i == 2:
            steps = mix(steps, lx)
        nw = len(lw) * NF // (NF + NC) if i < 4 else len(lw)
        wk = mix(work[:NF], lw[:nw]) if lw else work[:NF]
        if i == P - 1:
            phase(steps[:4], [])
            out_copy(0, P - 1)
            phase(steps[4:], [])
        else:
            phase(steps, wk)
        if STOP == i + 1:
            stop_here(1)
            return
        flush()
        dsteps = dn(i) if i != 4 else mix(dn(i), invs(P - 2) + invs(P - 1))
        phase(dsteps, mix(work[NF:], lw[nw:]) if lw[nw:] else work[NF:])
    flush()
    out_copy(P - 1, 1)
    for d in out_cps:
        d.wait()


@jax.jit
def pallas_adaLN_cond__ssm_conv_h3__glu_gated_bilinear__prompt_kernel(
    A_q, A_k, A_v, A_shift_k, A_ssm_k, A_ssm_D, B_x, B_w_gate, B_w_up, B_w_down, c, w_mod,
):
    del B_x
    hbm = pl.BlockSpec(memory_space=pl.ANY)
    out = pl.pallas_call(
        _kernel,
        in_specs=[hbm] * 11,
        out_specs=hbm,
        out_shape=jax.ShapeDtypeStruct((S, D), bf16),
        scratch_shapes=[
            pltpu.VMEM((S, D), bf16), pltpu.VMEM((S, D), bf16), pltpu.VMEM((S, D), bf16),
            pltpu.VMEM((D, S), bf16),
            pltpu.VMEM((1, D, F), bf16), pltpu.VMEM((1, D, F), bf16), pltpu.VMEM((1, F, D), bf16),
            pltpu.VMEM((D, 6 * D), bf16),
            pltpu.VMEM((L, N2), u32), pltpu.VMEM((N2, L), u32), pltpu.VMEM((L, L), u32),
            pltpu.VMEM((4, D), bf16), pltpu.VMEM((D,), bf16), pltpu.VMEM((1, D), bf16),
            pltpu.VMEM((P, 6, N2, D), f32),
            pltpu.VMEM((P, 6, N2, D), f32),
            pltpu.VMEM((4, N2, D), f32),
            pltpu.VMEM((P, 2, N2, D), u32),
            pltpu.VMEM((P, 2, N2 // 2, D), u32),
            pltpu.VMEM((P, L, D), f32),
            pltpu.VMEM((P, L, D), f32),
            pltpu.VMEM((P, N2, D), u32),
            pltpu.VMEM((2, N2, F), u32),
            pltpu.VMEM((S // 2, D), u32),
            pltpu.VMEM((L, D), f32),
            pltpu.SemaphoreType.DMA((64,)),
        ],
        compiler_params=pltpu.CompilerParams(vmem_limit_bytes=120 * 1024 * 1024),
    )(A_q.reshape(S, D), A_k.reshape(S, D), A_v.reshape(S, D), A_shift_k.T, A_ssm_k,
      A_ssm_D, B_w_gate, B_w_up, B_w_down, c, w_mod)
    return out.reshape(1, S, D)
```
